```python
import os as _os
_os.environ.setdefault("JAX_PLATFORMS", "cpu")
import jax
import jax.numpy as jnp

def _softmax(x, axis=-1):
    return jax.nn.softmax(x, axis=axis)
def _gelu(x):
    return jax.nn.gelu(x, approximate=True)
def _silu(x):
    return jax.nn.silu(x)
def _sigmoid(x):
    return jax.nn.sigmoid(x)
def _layernorm(x, axis=-1, eps=1e-5):
    m = jnp.mean(x, axis=axis, keepdims=True)
    v = jnp.var(x, axis=axis, keepdims=True)
    return (x - m) / jnp.sqrt(v + eps)
def _scatter_add(tgt, idx, src, axis=0):
    return tgt.at[idx].add(src)
def _segment_sum(src, seg, n):
    return jax.ops.segment_sum(src, seg, n)
class _Rng:
    def __init__(self, key):
        self._k = key
    def _next(self):
        self._k, sub = jax.random.split(self._k)
        return sub
    def normal(self, shape):
        return jax.random.normal(self._next(), shape, dtype=jnp.bfloat16)
    def randint(self, lo, hi, shape):
        return jax.random.randint(self._next(), shape, lo, hi, dtype=jnp.int32)
    def uniform(self, shape, lo=0.0, hi=1.0):
        return jax.random.uniform(self._next(), shape, jnp.bfloat16, lo, hi)
    def permutation(self, n):
        return jax.random.permutation(self._next(), n)


kernel_name = 'concat_heads__gqa_block_cached__gqa_block_cached__near_ridge'

def setup_inputs():
    _rng = _Rng(jax.random.key(int.from_bytes(__import__("os").urandom(4), "little")))
    _w = (lambda a: (lambda t: t.astype(jnp.bfloat16) if jnp.issubdtype(t.dtype, jnp.floating) else t)(jnp.asarray(a)))
    def _A_setup():
        B, Sq, D = 8, 128, 576
        Hq, Hkv, Sk, Dh = 32, 16, 512, 128
        assert Hq % Hkv == 0, (Hq, Hkv)
        return {
            "x": _w((lambda *s: _rng.normal(s) * 0.8)(B, Sq, D)),
            "k_cache": _w((lambda *s: _rng.normal(s) * 0.8)(B, Hkv, Sk, Dh)),
            "v_cache": _w((lambda *s: _rng.normal(s) * 0.05)(B, Hkv, Sk, Dh)),
            "wq": _w((lambda *s: _rng.normal(s) * 0.8)(D, Hq * Dh) * (D ** -0.5)),
            "wo": _w((lambda *s: _rng.normal(s) * 0.05)(Hq * Dh, D) * ((Hq * Dh) ** -0.5)),
        }
    _A_in = _A_setup()

    def _B_setup():
        B, Sq, D = 8, 128, 576
        Hq, Hkv, Sk, Dh = 32, 16, 512, 128
        assert Hq % Hkv == 0, (Hq, Hkv)
        return {
            "x": _w((lambda *s: _rng.normal(s) * 0.8)(B, Sq, D)),
            "k_cache": _w((lambda *s: _rng.normal(s) * 0.8)(B, Hkv, Sk, Dh)),
            "v_cache": _w((lambda *s: _rng.normal(s) * 0.05)(B, Hkv, Sk, Dh)),
            "wq": _w((lambda *s: _rng.normal(s) * 0.8)(D, Hq * Dh) * (D ** -0.5)),
            "wo": _w((lambda *s: _rng.normal(s) * 0.05)(Hq * Dh, D) * ((Hq * Dh) ** -0.5)),
        }
    _B_in = _B_setup()

    return {
        "A_x": _A_in["x"],
        "A_k_cache": _A_in["k_cache"],
        "A_v_cache": _A_in["v_cache"],
        "A_wq": _A_in["wq"],
        "A_wo": _A_in["wo"],
        "B_x": _B_in["x"],
        "B_k_cache": _B_in["k_cache"],
        "B_v_cache": _B_in["v_cache"],
        "B_wq": _B_in["wq"],
        "B_wo": _B_in["wo"],
    }

def reference(A_x, A_k_cache, A_v_cache, A_wq, A_wo, B_x, B_k_cache, B_v_cache, B_wq, B_wo):
    def _A_ref(x, k_cache, v_cache, wq, wo):
        B, Sq, D = x.shape
        Hq, Dh = 32, 128
        Hkv = k_cache.shape[1]
        rep = Hq // Hkv
        q = (lambda x, *d: x.transpose(*d))((x @ wq).reshape(B, Sq, Hq, Dh), 0, 2, 1, 3)
        k = jnp.repeat(k_cache, rep, axis=1)
        v = jnp.repeat(v_cache, rep, axis=1)
        scores = jnp.einsum("bhqd,bhkd->bhqk", q, k) * (Dh ** -0.5)
        p = _softmax(scores, axis=-1)
        o = jnp.einsum("bhqk,bhkd->bhqd", p, v)
        return (lambda x, *d: x.transpose(*d))(o, 0, 2, 1, 3).reshape(B, Sq, Hq * Dh) @ wo

    def _B_ref(x, k_cache, v_cache, wq, wo):
        B, Sq, D = x.shape
        Hq, Dh = 32, 128
        Hkv = k_cache.shape[1]
        rep = Hq // Hkv
        q = (lambda x, *d: x.transpose(*d))((x @ wq).reshape(B, Sq, Hq, Dh), 0, 2, 1, 3)
        k = jnp.repeat(k_cache, rep, axis=1)
        v = jnp.repeat(v_cache, rep, axis=1)
        scores = jnp.einsum("bhqd,bhkd->bhqk", q, k) * (Dh ** -0.5)
        p = _softmax(scores, axis=-1)
        o = jnp.einsum("bhqk,bhkd->bhqd", p, v)
        return (lambda x, *d: x.transpose(*d))(o, 0, 2, 1, 3).reshape(B, Sq, Hq * Dh) @ wo

    a = _A_ref(A_x, A_k_cache, A_v_cache, A_wq, A_wo)
    b = _B_ref(B_x, B_k_cache, B_v_cache, B_wq, B_wo)
    return jnp.concatenate([a, b], axis=-1)
```

```python
import jax
import jax.numpy as jnp
import jax.experimental.pallas as pl
import jax.experimental.pallas.tpu as pltpu

B, SQ, D = 8, 128, 576
HQ, HKV, SK, DH = 32, 16, 512, 128
REP = HQ // HKV
G = 4
NG = HKV // G
GW = G * REP * DH
PW = GW // B
T = NG * B
LOG2E = 1.4426950408889634
QSCALE = (DH ** -0.5) * LOG2E
NT = (((1,), (1,)), ((), ()))
TN = (((0,), (0,)), ((), ()))


def _qproj(xt, wq):
    q = jax.lax.dot_general(xt, wq, TN, preferred_element_type=jnp.float32)
    return (q * QSCALE).astype(jnp.bfloat16)


def _attn_oproj(q, k_ref, v_ref, wot):
    outs = []
    for j in range(G):
        q2 = jnp.concatenate(
            [q[:, (2 * j) * DH:(2 * j + 1) * DH], q[:, (2 * j + 1) * DH:(2 * j + 2) * DH]], axis=0)
        s = jax.lax.dot_general(q2, k_ref[j], NT, preferred_element_type=jnp.float32)
        m = jnp.max(s, axis=-1, keepdims=True)
        p = jnp.exp2(s - m)
        l = jnp.sum(p, axis=-1, keepdims=True)
        o = jnp.dot(p.astype(jnp.bfloat16), v_ref[j], preferred_element_type=jnp.float32)
        r = pl.reciprocal(l, approx=True)
        r = r * (2.0 - l * r)
        o = o * r
        outs += [o[:SQ], o[SQ:]]
    o_cat = jnp.concatenate(outs, axis=1).astype(jnp.bfloat16)
    return jax.lax.dot_general(wot, o_cat, NT, preferred_element_type=jnp.float32)


def _kernel(xa_h, ka_h, va_h, wqa_h, woa_h, xb_h, kb_h, vb_h, wqb_h, wob_h, out_h,
            x_v, kv_v, w_v, q_v, acc, ostage, x_sem, kv_sem, w_sem, o_sem):
    kv_h = (ka_h, va_h, kb_h, vb_h)
    w_h = (wqa_h, wqb_h, woa_h, wob_h)
    x_h = (xa_h, xb_h)

    def kv_copy(gg, bb, sl, i):
        return pltpu.make_async_copy(kv_h[i].at[bb, pl.ds(gg * G, G)], kv_v.at[sl, i], kv_sem.at[sl, i])

    def w_piece(gg, i, p):
        return pltpu.make_async_copy(w_h[i].at[:, pl.ds(gg * GW + p * PW, PW)],
                                     w_v.at[gg, i, :, pl.ds(p * PW, PW)], w_sem.at[gg, i])

    def w_full(gg, i):
        return pltpu.make_async_copy(w_h[i].at[:, pl.ds(gg * GW, GW)], w_v.at[gg, i], w_sem.at[gg, i])

    def x_copy(bb, i):
        return pltpu.make_async_copy(x_h[i].at[bb], x_v.at[i, bb], x_sem.at[i, bb])

    def o_copy(bb):
        return pltpu.make_async_copy(ostage.at[bb % 2], out_h.at[bb], o_sem.at[bb % 2])

    x_copy(0, 0).start()
    w_full(0, 0).start()
    x_copy(0, 0).wait()
    w_full(0, 0).wait()
    for bb in range(1, B):
        x_copy(bb, 0).start()
    w_full(0, 1).start()
    for bb in range(B):
        x_copy(bb, 1).start()
    for i in range(4):
        kv_copy(0, 0, 0, i).start()
    for i in range(2, 4):
        w_full(0, i).start()
    if NG > 1:
        for i in range(2):
            w_full(1, i).start()
    for bb in range(B):
        if bb > 0:
            x_copy(bb, 0).wait()
        q_v[0, bb] = _qproj(x_v[0, bb], w_v[0, 0])
    w_full(0, 1).wait()
    for bb in range(B):
        x_copy(bb, 1).wait()
        q_v[1, bb] = _qproj(x_v[1, bb], w_v[0, 1])

    def body(t, last):
        g = t // B
        b = t % B
        slot = t % 2
        t1 = t + 1
        g1 = t1 // B
        b1 = t1 % B
        for i in range(4):
            kv_copy(g, b, slot, i).wait()

        @pl.when(b == 0)
        def _():
            for i in range(2, 4):
                w_full(g, i).wait()
            if not last:
                for i in range(2):
                    w_full(g + 1, i).wait()

        if last:
            @pl.when(b >= 2)
            def _():
                o_copy(b - 2).wait()

        if last:
            @pl.when(t1 < T)
            def _():
                for i in range(4):
                    kv_copy(g1, b1, 1 - slot, i).start()
        else:
            for i in range(4):
                kv_copy(g1, b1, 1 - slot, i).start()
            for i in range(2, 4):
                w_piece(g + 1, i, b).start()

            @pl.when(g + 2 < NG)
            def _():
                for i in range(2):
                    w_piece(g + 2, i, b).start()

        qa = q_v[0, b]
        qb = q_v[1, b]
        ca = _attn_oproj(qa, kv_v.at[slot, 0], kv_v.at[slot, 1], w_v[g, 2])
        cb = _attn_oproj(qb, kv_v.at[slot, 2], kv_v.at[slot, 3], w_v[g, 3])
        c = jnp.concatenate([ca, cb], axis=0)
        if last:
            cn = acc[b] + c if NG > 1 else c
            ostage[b % 2] = cn.T.astype(ostage.dtype)
            o_copy(b).start()
        else:
            acc[b] = jnp.where(g == 0, c, acc[b] + c)
            q_v[0, b] = _qproj(x_v[0, b], w_v[g + 1, 0])
            q_v[1, b] = _qproj(x_v[1, b], w_v[g + 1, 1])

    def loop1(t, carry):
        body(t, False)
        return carry

    def loop2(t, carry):
        body(t, True)
        return carry

    jax.lax.fori_loop(0, T - B, loop1, 0)
    jax.lax.fori_loop(T - B, T, loop2, 0)
    o_copy(B - 2).wait()
    o_copy(B - 1).wait()


@jax.jit
def pallas_concat_heads__gqa_block_cached__gqa_block_cached__near_ridge_kernel(
        A_x, A_k_cache, A_v_cache, A_wq, A_wo, B_x, B_k_cache, B_v_cache, B_wq, B_wo):
    any_spec = pl.BlockSpec(memory_space=pl.ANY)
    return pl.pallas_call(
        _kernel,
        in_specs=[any_spec] * 10,
        out_specs=any_spec,
        out_shape=jax.ShapeDtypeStruct((B, SQ, 2 * D), jnp.bfloat16),
        scratch_shapes=[
            pltpu.VMEM((2, B, D, SQ), jnp.bfloat16),
            pltpu.VMEM((2, 4, G, SK, DH), jnp.bfloat16),
            pltpu.VMEM((NG, 4, D, GW), jnp.bfloat16),
            pltpu.VMEM((2, B, SQ, GW), jnp.bfloat16),
            pltpu.VMEM((B, 2 * D, SQ), jnp.float32),
            pltpu.VMEM((2, SQ, 2 * D), jnp.bfloat16),
            pltpu.SemaphoreType.DMA((2, B)),
            pltpu.SemaphoreType.DMA((2, 4)),
            pltpu.SemaphoreType.DMA((NG, 4)),
            pltpu.SemaphoreType.DMA((2,)),
        ],
        compiler_params=pltpu.CompilerParams(
            vmem_limit_bytes=96 * 1024 * 1024,
            disable_bounds_checks=True),
    )(jnp.swapaxes(A_x, 1, 2), A_k_cache, A_v_cache, A_wq, A_wo.T,
      jnp.swapaxes(B_x, 1, 2), B_k_cache, B_v_cache, B_wq, B_wo.T)
```

```python
import jax
import jax.numpy as jnp
import jax.experimental.pallas as pl
import jax.experimental.pallas.tpu as pltpu

B, SQ, D = 8, 128, 576
HQ, HKV, SK, DH = 32, 16, 512, 128
REP = HQ // HKV
G = 8
NG = HKV // G
GW = G * REP * DH
PW = GW // B
C0 = 512
B0 = 2
LOG2E = 1.4426950408889634
QSCALE = (DH ** -0.5) * LOG2E
NT = (((1,), (1,)), ((), ()))


def _qproj(x, wq):
    q = jnp.dot(x, wq, preferred_element_type=jnp.float32)
    return (q * QSCALE).astype(jnp.bfloat16)


def _attn_oproj(qs, krefs, vrefs, wots):
    outs = ([], [])
    for j in range(G):
        ss = []
        for br in range(2):
            q = qs[br]
            q2 = jnp.concatenate(
                [q[:, (2 * j) * DH:(2 * j + 1) * DH], q[:, (2 * j + 1) * DH:(2 * j + 2) * DH]], axis=0)
            ss.append(jax.lax.dot_general(q2, krefs[br][j], NT, preferred_element_type=jnp.float32))
        for br in range(2):
            s = ss[br]
            m = jnp.max(s, axis=-1, keepdims=True)
            p = jnp.exp2(s - m)
            l = jnp.sum(p, axis=-1, keepdims=True)
            o = jnp.dot(p.astype(jnp.bfloat16), vrefs[br][j], preferred_element_type=jnp.float32)
            r = pl.reciprocal(l, approx=True)
            r = r * (2.0 - l * r)
            o = o * r
            outs[br].extend([o[:SQ], o[SQ:]])
    cs = []
    for br in range(2):
        o_cat = jnp.concatenate(outs[br], axis=1).astype(jnp.bfloat16)
        cs.append(jax.lax.dot_general(wots[br], o_cat, NT, preferred_element_type=jnp.float32))
    return jnp.concatenate(cs, axis=0)


def _kernel(xa_h, ka_h, va_h, wqa_h, woa_h, xb_h, kb_h, vb_h, wqb_h, wob_h, out_h,
            x_v, xs, kv_v, w_v, q_v, acc, ostage, x_sem, kv_sem, w_sem, o_sem):
    kv_h = (ka_h, va_h, kb_h, vb_h)
    w_h = (wqa_h, wqb_h, woa_h, wob_h)
    x_h = (xa_h, xb_h)

    def kv_copy(gg, bb, sl, i):
        return pltpu.make_async_copy(kv_h[i].at[bb, pl.ds(gg * G, G)], kv_v.at[sl, i], kv_sem.at[sl, i])

    def w_piece(gg, i, p):
        return pltpu.make_async_copy(w_h[i].at[:, pl.ds(gg * GW + p * PW, PW)],
                                     w_v.at[gg, i, :, pl.ds(p * PW, PW)], w_sem.at[gg, i])

    def w_full(gg, i):
        return pltpu.make_async_copy(w_h[i].at[:, pl.ds(gg * GW, GW)], w_v.at[gg, i], w_sem.at[gg, i])

    def x_copy(lo, n, i, s):
        return pltpu.make_async_copy(x_h[i].at[pl.ds(lo, n)], x_v.at[i, pl.ds(lo, n)], x_sem.at[s])

    def o_copy(bb):
        return pltpu.make_async_copy(ostage.at[bb % 2], out_h.at[bb], o_sem.at[bb % 2])

    def wq0_copy(part):
        lo, n = (0, C0) if part == 0 else (C0, GW - C0)
        return pltpu.make_async_copy(w_h[0].at[:, pl.ds(lo, n)], w_v.at[0, 0, :, pl.ds(lo, n)],
                                     x_sem.at[3 + part])

    def q_units(br, bbs, lo, hi, first):
        for bb in bbs:
            if first:
                x = x_v[br, bb].T
                xs[br, bb] = x
            else:
                x = xs[br, bb]
            q_v[br, bb, :, lo:hi] = _qproj(x, w_v[0, br, :, lo:hi])

    x_copy(0, B0, 0, 0).start()
    wq0_copy(0).start()
    x_copy(0, B0, 0, 0).wait()
    wq0_copy(0).wait()
    x_copy(B0, B - B0, 0, 1).start()
    wq0_copy(1).start()
    q_units(0, range(B0), 0, C0, True)
    x_copy(B0, B - B0, 0, 1).wait()
    w_full(0, 1).start()
    x_copy(0, B, 1, 2).start()
    for i in range(4):
        kv_copy(0, 0, 0, i).start()
    for i in range(2, 4):
        w_full(0, i).start()
    if NG > 1:
        for i in range(2):
            w_full(1, i).start()
    q_units(0, range(B0, B), 0, C0, True)
    wq0_copy(1).wait()
    q_units(0, range(B), C0, GW, False)
    w_full(0, 1).wait()
    x_copy(0, B, 1, 2).wait()
    q_units(1, range(B), 0, GW, True)

    for g in range(NG):
        last = g == NG - 1
        for i in range(2, 4):
            w_full(g, i).wait()
        if not last:
            for i in range(2):
                w_full(g + 1, i).wait()

        def body(b, carry, g=g, last=last):
            slot = b % 2
            for i in range(4):
                kv_copy(g, b, slot, i).wait()
            if last:
                @pl.when(b >= 2)
                def _():
                    o_copy(b - 2).wait()

                @pl.when(b + 1 < B)
                def _():
                    for i in range(4):
                        kv_copy(g, b + 1, 1 - slot, i).start()
            else:
                wrap = (b + 1) // B
                for i in range(4):
                    kv_copy(g + wrap, (b + 1) % B, 1 - slot, i).start()
                for i in range(2, 4):
                    w_piece(g + 1, i, b).start()
                if g + 2 < NG:
                    for i in range(2):
                        w_piece(g + 2, i, b).start()
                qn = [_qproj(xs[br, b], w_v[g + 1, br]) for br in range(2)]

            qs = [q_v[br, b] for br in range(2)]
            c = _attn_oproj(qs, [kv_v.at[slot, 0], kv_v.at[slot, 2]], [kv_v.at[slot, 1], kv_v.at[slot, 3]],
                            [w_v[g, 2], w_v[g, 3]])
            if g > 0:
                c = acc[b] + c
            if last:
                ostage[slot] = c.T.astype(ostage.dtype)
                o_copy(b).start()
            else:
                acc[b] = c
                for br in range(2):
                    q_v[br, b] = qn[br]
            return carry

        jax.lax.fori_loop(0, B, body, 0)
    o_copy(B - 2).wait()
    o_copy(B - 1).wait()


@jax.jit
def pallas_concat_heads__gqa_block_cached__gqa_block_cached__near_ridge_kernel(
        A_x, A_k_cache, A_v_cache, A_wq, A_wo, B_x, B_k_cache, B_v_cache, B_wq, B_wo):
    any_spec = pl.BlockSpec(memory_space=pl.ANY)
    return pl.pallas_call(
        _kernel,
        in_specs=[any_spec] * 10,
        out_specs=any_spec,
        out_shape=jax.ShapeDtypeStruct((B, SQ, 2 * D), jnp.bfloat16),
        scratch_shapes=[
            pltpu.VMEM((2, B, D, SQ), jnp.bfloat16),
            pltpu.VMEM((2, B, SQ, D), jnp.bfloat16),
            pltpu.VMEM((2, 4, G, SK, DH), jnp.bfloat16),
            pltpu.VMEM((NG, 4, D, GW), jnp.bfloat16),
            pltpu.VMEM((2, B, SQ, GW), jnp.bfloat16),
            pltpu.VMEM((B, 2 * D, SQ), jnp.float32),
            pltpu.VMEM((2, SQ, 2 * D), jnp.bfloat16),
            pltpu.SemaphoreType.DMA((5,)),
            pltpu.SemaphoreType.DMA((2, 4)),
            pltpu.SemaphoreType.DMA((NG, 4)),
            pltpu.SemaphoreType.DMA((2,)),
        ],
        compiler_params=pltpu.CompilerParams(
            vmem_limit_bytes=96 * 1024 * 1024,
            disable_bounds_checks=True),
    )(jnp.swapaxes(A_x, 1, 2), A_k_cache, A_v_cache, A_wq, A_wo.T,
      jnp.swapaxes(B_x, 1, 2), B_k_cache, B_v_cache, B_wq, B_wo.T)
```
